```python
import os as _os
_os.environ.setdefault('JAX_PLATFORMS', 'cpu')
import jax
import jax.numpy as jnp

def _softmax(x, axis=-1):
    return jax.nn.softmax(x, axis=axis)

def _gelu(x):
    return jax.nn.gelu(x, approximate=True)

def _silu(x):
    return jax.nn.silu(x)

def _sigmoid(x):
    return jax.nn.sigmoid(x)

def _layernorm(x, axis=-1, eps=1e-05):
    m = jnp.mean(x, axis=axis, keepdims=True)
    v = jnp.var(x, axis=axis, keepdims=True)
    return (x - m) / jnp.sqrt(v + eps)

def _scatter_add(tgt, idx, src, axis=0):
    return tgt.at[idx].add(src)

def _segment_sum(src, seg, n):
    return jax.ops.segment_sum(src, seg, n)

class _Rng:

    def __init__(self, key):
        self._k = key

    def _next(self):
        self._k, sub = jax.random.split(self._k)
        return sub

    def normal(self, shape):
        return jax.random.normal(self._next(), shape, dtype=jnp.bfloat16)

    def randint(self, lo, hi, shape):
        return jax.random.randint(self._next(), shape, lo, hi, dtype=jnp.int32)

    def uniform(self, shape, lo=0.0, hi=1.0):
        return jax.random.uniform(self._next(), shape, jnp.bfloat16, lo, hi)

    def permutation(self, n):
        return jax.random.permutation(self._next(), n)
kernel_name = 'interleave_layers__memory_aug_recurrent_mem_tr__mixer_token_mlp__prompt'

def setup_inputs():
    _rng = _Rng(jax.random.key(int.from_bytes(__import__("os").urandom(4), "little")))
    _w = lambda a: (lambda t: t.astype(jnp.bfloat16) if jnp.issubdtype(t.dtype, jnp.floating) else t)(jnp.asarray(a))

    def _A_setup():
        B, S, Dm = (1, 2048, 640)
        H, Dh = (32, 128)
        M, seg = (8, 32)
        seg = min(seg, S)
        S = S // seg * seg
        return {'x': _w((lambda *s: _rng.normal(s) * 0.05)(B, S, Dm)), 'mem0': _w((lambda *s: _rng.normal(s) * 0.2)(B, M, Dm)), 'Wq': _w((lambda *s: _rng.normal(s) * 0.8)(Dm, H, Dh) * Dm ** (-0.5)), 'Wk': _w((lambda *s: _rng.normal(s) * 0.8)(Dm, H, Dh) * Dm ** (-0.5)), 'Wv': _w((lambda *s: _rng.normal(s) * 0.2)(Dm, H, Dh) * Dm ** (-0.5)), 'Wo': _w((lambda *s: _rng.normal(s) * 0.2)(H, Dh, Dm) * (H * Dh) ** (-0.5)), 'seg_len': seg}
    _A_in = _A_setup()

    def _B_setup():
        B, S, D, F = (1, 2048, 640, 1728)
        return {'x': _w((lambda *s: _rng.normal(s) * 0.05)(B, S, D)), 'w1': _w((lambda *s: _rng.normal(s) * 0.2)(S, F) * S ** (-0.5)), 'b1': _w((lambda *s: _rng.normal(s) * 0.2)(F) * 0.02), 'w2': _w((lambda *s: _rng.normal(s) * 0.2)(F, S) * F ** (-0.5)), 'b2': _w((lambda *s: _rng.normal(s) * 0.2)(S) * 0.02)}
    _B_in = _B_setup()
    return {'A_x': _A_in['x'], 'A_mem0': _A_in['mem0'], 'A_Wq': _A_in['Wq'], 'A_Wk': _A_in['Wk'], 'A_Wv': _A_in['Wv'], 'A_Wo': _A_in['Wo'], 'A_seg_len': _A_in['seg_len'], 'B_x': _B_in['x'], 'B_w1': _B_in['w1'], 'B_b1': _B_in['b1'], 'B_w2': _B_in['w2'], 'B_b2': _B_in['b2']}

def reference(A_x, A_mem0, A_Wq, A_Wk, A_Wv, A_Wo, A_seg_len, B_x, B_w1, B_b1, B_w2, B_b2):

    def _A_ref(x, mem0, Wq, Wk, Wv, Wo, seg_len):
        B, S, Dm = x.shape
        H, Dh = (Wq.shape[1], Wq.shape[2])
        M = mem0.shape[1]
        scale = Dh ** (-0.5)
        n_seg = S // seg_len
        L = M + seg_len
        idx = jnp.arange(L)
        mask = (idx[:, None] < M) | (idx[:, None] >= idx[None, :])
        mem = mem0
        outs = []
        for s in range(n_seg):
            xs = x[:, s * seg_len:(s + 1) * seg_len, :].copy()
            h = jnp.concatenate([mem, xs], axis=1)
            q = jnp.einsum('btd,dhe->bhte', h, Wq)
            k = jnp.einsum('btd,dhe->bhte', h, Wk)
            v = jnp.einsum('btd,dhe->bhte', h, Wv)
            scores = jnp.einsum('bhqe,bhke->bhqk', q, k) * scale
            scores = jnp.where(mask[None, None], scores, -1000000000.0)
            p = _softmax(scores, axis=-1)
            o = jnp.einsum('bhqk,bhke->bhqe', p, v)
            o = jnp.einsum('bhte,hed->btd', o, Wo)
            mem = o[:, :M, :].copy()
            outs.append(o[:, M:, :])
        return jnp.concatenate(outs, axis=1)

    def _B_ref(x, w1, b1, w2, b2):
        B, S, D = x.shape
        h = _layernorm(x, axis=-1)
        u = jnp.einsum('bsd,sf->bdf', h, w1) + b1
        u = _gelu(u)
        y = jnp.einsum('bdf,fs->bds', u, w2) + b2
        return (lambda x, *d: x.transpose(*d))(y, 0, 2, 1)
    x = A_x
    x = x + _A_ref(_layernorm(x, axis=-1), A_mem0, A_Wq, A_Wk, A_Wv, A_Wo, A_seg_len)
    x = x + _B_ref(_layernorm(x, axis=-1), B_w1, B_b1, B_w2, B_b2)
    x = x + _A_ref(_layernorm(x, axis=-1), A_mem0, A_Wq, A_Wk, A_Wv, A_Wo, A_seg_len)
    x = x + _B_ref(_layernorm(x, axis=-1), B_w1, B_b1, B_w2, B_b2)
    return x
```

```python
import functools

import jax
import jax.numpy as jnp
import numpy as np
from jax import lax
import jax.experimental.pallas as pl
import jax.experimental.pallas.tpu as pltpu

_LANES = 128
_EPS = 1e-5
_LOG2E = float(np.log2(np.e))
_NN = (((1,), (0,)), ((), ()))
_NT = (((1,), (1,)), ((), ()))
_TN = (((0,), (0,)), ((), ()))
_F32 = jnp.float32
_BF16 = jnp.bfloat16

CFG = dict(ds=2, dpv=6, do_first=0, m1=192, m2=128, nlayers=2, skip_b=False)


def _dot(a, b, dims=_NN):
    return lax.dot_general(a, b, dims, preferred_element_type=_F32)


def _layernorm(x):
    inv_d = 1.0 / x.shape[-1]
    m = jnp.sum(x, axis=-1, keepdims=True) * inv_d
    c = x - m
    v = jnp.sum(c * c, axis=-1, keepdims=True) * inv_d
    return c * lax.rsqrt(v + _EPS)


def _gelu(x):
    c = float(np.sqrt(2.0 / np.pi))
    return 0.5 * x * (1.0 + jnp.tanh(c * (x + 0.044715 * (x * x * x))))


def _column(row):
    return jnp.broadcast_to(row, (_LANES, row.shape[1])).T


def _kernel(x_hbm, mem0_ref, wq_hbm, wk_hbm, wv_hbm, wo_hbm, w1t_hbm, b1_ref, w2_hbm, b2_ref,
            out_hbm,
            xio_ref, xs_ref, xn_ref, hb_ref, stage_ref, wqkv_ref, wo_ref, w1t_ref, w2_ref,
            g_ref, b1c_ref, b2c_ref, h_ref, e_ref, r_ref, o_ref, sems,
            *, seg, cfg):
    S, D = xs_ref.shape
    M = mem0_ref.shape[0]
    L = seg + M
    H = wqkv_ref.shape[1]
    Dh = wqkv_ref.shape[3]
    F = w1t_ref.shape[0]
    n_seg = S // seg
    nd = D // _LANES
    n_pairs = H // 2

    x_cp = pltpu.make_async_copy(x_hbm, xio_ref, sems.at[0])
    x_cp.start()
    w_cps = []
    for i, w in enumerate((wq_hbm, wk_hbm, wv_hbm)):
        wu = w.bitcast(jnp.uint32)
        for p in range(n_pairs):
            j = i * n_pairs + p
            w_cps.append(pltpu.make_async_copy(wu.at[:, p, :], stage_ref.at[j], sems.at[8 + j]))
    for c in w_cps:
        c.start()
    wo_cps = [pltpu.make_async_copy(wo_hbm.at[:, pl.ds(j * _LANES, _LANES)], wo_ref.at[j], sems.at[1 + j])
              for j in range(nd)]
    for c in wo_cps:
        c.start()
    w1_cp = pltpu.make_async_copy(w1t_hbm, w1t_ref, sems.at[6])
    w2_cp = pltpu.make_async_copy(w2_hbm, w2_ref, sems.at[7])

    b1c_ref[...] = _column(b1_ref[...].astype(_F32))
    b2c_ref[...] = _column(b2_ref[...].astype(_F32))

    x_cp.wait()
    RB = 128

    def ln0(i, c):
        rows = pl.ds(pl.multiple_of(i * RB, RB), RB)
        x = xio_ref[rows, :].astype(_F32)
        xs_ref[rows, :] = x
        xn_ref[rows, :] = _layernorm(x)
        return c

    with jax.named_scope('ln0'):
        lax.fori_loop(0, S // RB, ln0, 0)

    for j, c in enumerate(w_cps):
        c.wait()
        i, p = divmod(j, n_pairs)
        u = stage_ref[j]
        for b in range(2):
            w = pltpu.unpack_elementwise(u, index=b, packed_dtype=_BF16, unpacked_dtype=_F32)
            wqkv_ref[i, 2 * p + b] = w.astype(_BF16)
    for c in wo_cps:
        c.wait()
    w1_cp.start()
    w2_cp.start()

    qk_scale = float(Dh) ** -0.5 * _LOG2E

    def a_step(s, carry):
        rows = pl.ds(pl.multiple_of(s * seg, seg), seg)
        h_ref[0:seg, :] = xn_ref[rows, :]
        row = lax.broadcasted_iota(jnp.int32, (L, _LANES), 0)
        col = lax.broadcasted_iota(jnp.int32, (L, _LANES), 1)
        visible = ((col <= row) | (col >= seg) | (row >= seg)) & (col < L)
        fill = jnp.where(col < L, -1e9 * _LOG2E, -jnp.inf).astype(_F32)
        zpad = jnp.zeros((_LANES - L - 8, Dh), _BF16)

        def pad_rhs(t):
            t = jnp.concatenate([t, jnp.zeros((8, Dh), _F32)], axis=0).astype(_BF16)
            return jnp.concatenate([t, zpad], axis=0)

        q = {}
        k = {}
        v = {}

        def op_qk(h):
            q[h] = _dot(h_ref[...], wqkv_ref[0, h])
            k[h] = pad_rhs(_dot(h_ref[...], wqkv_ref[1, h]))

        def op_s(h):
            sc = _dot(q.pop(h), k.pop(h), _NT)
            t = jnp.where(visible, sc * qk_scale, fill)
            e = jnp.exp2(t - jnp.max(t, axis=-1, keepdims=True))
            e_ref[h] = e
            r_ref[h] = jnp.broadcast_to(1.0 / jnp.sum(e, axis=-1, keepdims=True), (L, Dh))

        def op_v(h):
            v[h] = pad_rhs(_dot(h_ref[...], wqkv_ref[2, h]))

        def op_pv(h):
            o_ref[:, h * Dh:(h + 1) * Dh] = _dot(e_ref[h], v.pop(h)) * r_ref[h]

        ds, dpv = cfg["ds"], cfg["dpv"]
        for i in range(H):
            op_qk(i)
            if i - ds >= 0:
                op_s(i - ds)
        for i in range(H):
            op_v(i)
            if H - ds + i < H:
                op_s(H - ds + i)
            if i - dpv >= 0:
                op_pv(i - dpv)
        split = (H - dpv - 8) * Dh
        acc0 = _dot(o_ref[:, 0:split], wo_ref[0, 0:split, :])
        for i in range(H - dpv, H):
            op_pv(i)
        acc1 = _dot(o_ref[:, 0:split], wo_ref[1, 0:split, :])
        for j in range(nd):
            cols = slice(j * _LANES, (j + 1) * _LANES)
            if j == 0:
                y = acc0 + _dot(o_ref[:, split:], wo_ref[0, split:, :])
            elif j == 1:
                y = acc1 + _dot(o_ref[:, split:], wo_ref[1, split:, :])
            else:
                y = _dot(o_ref[...], wo_ref[j])
            h_ref[seg:L, cols] = y[seg:L]
            xs_ref[rows, cols] = xs_ref[rows, cols] + y[0:seg]
        return carry

    def layer(l, carry):
        h_ref[seg:L, :] = mem0_ref[...].astype(_F32)
        with jax.named_scope('A'):
            lax.fori_loop(0, n_seg, a_step, 0)

        @pl.when(l == 0)
        def _():
            w1_cp.wait()
            w2_cp.wait()

        if cfg["skip_b"]:
            return carry

        def ln2(i, c):
            rows = pl.ds(pl.multiple_of(i * RB, RB), RB)
            hb_ref[rows, :] = _layernorm(_layernorm(xs_ref[rows, :])).astype(_BF16)
            return c

        with jax.named_scope('ln2'):
            lax.fori_loop(0, S // RB, ln2, 0)

        m1 = cfg["m1"]

        def up(i, c):
            rows = pl.ds(pl.multiple_of(i * m1, m1), m1)
            u = _dot(w1t_ref[rows, :], hb_ref[...])
            b = b1c_ref[rows, :]
            for j in range(nd):
                cols = slice(j * _LANES, (j + 1) * _LANES)
                g_ref[rows, cols] = _gelu(u[:, cols] + b).astype(_BF16)
            return c

        with jax.named_scope('up'):
            lax.fori_loop(0, F // m1, up, 0)

        m2 = cfg["m2"]

        def down(i, c):
            rows = pl.ds(pl.multiple_of(i * m2, m2), m2)
            y = _dot(w2_ref[:, rows], g_ref[...], _TN)
            b = b2c_ref[rows, :]
            x = xs_ref[rows, :] + (y + jnp.concatenate([b] * nd, axis=1))
            xs_ref[rows, :] = x
            xn_ref[rows, :] = _layernorm(x)
            xio_ref[rows, :] = x.astype(_BF16)
            return c

        with jax.named_scope('down'):
            lax.fori_loop(0, S // m2, down, 0)
        return carry

    lax.fori_loop(0, cfg["nlayers"], layer, 0)
    out_cp = pltpu.make_async_copy(xio_ref, out_hbm, sems.at[0])
    out_cp.start()
    out_cp.wait()


def build(cfg, A_x, A_mem0, A_Wq, A_Wk, A_Wv, A_Wo, B_w1, B_b1, B_w2, B_b2, seg=32):
    _, S, D = A_x.shape
    M = A_mem0.shape[1]
    H, Dh = A_Wq.shape[1], A_Wq.shape[2]
    F = B_w1.shape[1]
    L = seg + M
    hbm = pl.BlockSpec(memory_space=pltpu.HBM)
    vmem = pl.BlockSpec(memory_space=pltpu.VMEM)
    out = pl.pallas_call(
        functools.partial(_kernel, seg=seg, cfg=cfg),
        out_shape=jax.ShapeDtypeStruct((S, D), A_x.dtype),
        in_specs=[hbm, vmem, hbm, hbm, hbm, hbm, hbm, vmem, hbm, vmem],
        out_specs=hbm,
        scratch_shapes=[
            pltpu.VMEM((S, D), _BF16),
            pltpu.VMEM((S, D), _F32),
            pltpu.VMEM((S, D), _F32),
            pltpu.VMEM((S, D), _BF16),
            pltpu.VMEM((3 * H // 2, D, Dh), jnp.uint32),
            pltpu.VMEM((3, H, D, Dh), _BF16),
            pltpu.VMEM((D // _LANES, H * Dh, _LANES), _BF16),
            pltpu.VMEM((F, S), _BF16),
            pltpu.VMEM((F, S), _BF16),
            pltpu.VMEM((F, D), _BF16),
            pltpu.VMEM((F, _LANES), _F32),
            pltpu.VMEM((S, _LANES), _F32),
            pltpu.VMEM((L, D), _F32),
            pltpu.VMEM((H, L, _LANES), _F32),
            pltpu.VMEM((H, L, Dh), _F32),
            pltpu.VMEM((L, H * Dh), _F32),
            pltpu.SemaphoreType.DMA((8 + 3 * H // 2,)),
        ],
        compiler_params=pltpu.CompilerParams(vmem_limit_bytes=110 * 1024 * 1024),
        name="fused",
    )(A_x.reshape(S, D), A_mem0.reshape(M, D), A_Wq, A_Wk, A_Wv, A_Wo.reshape(H * Dh, D),
      B_w1.T, B_b1.reshape(1, F), B_w2, B_b2.reshape(1, S))
    return out.reshape(A_x.shape)


@functools.partial(jax.jit, static_argnames=("A_seg_len",))
def pallas_interleave_layers__memory_aug_recurrent_mem_tr__mixer_token_mlp__prompt_kernel(
    A_x: jax.Array,
    A_mem0: jax.Array,
    A_Wq: jax.Array,
    A_Wk: jax.Array,
    A_Wv: jax.Array,
    A_Wo: jax.Array,
    A_seg_len: int,
    B_x: jax.Array,
    B_w1: jax.Array,
    B_b1: jax.Array,
    B_w2: jax.Array,
    B_b2: jax.Array,
):
    del B_x
    return build(CFG, A_x, A_mem0, A_Wq, A_Wk, A_Wv, A_Wo, B_w1, B_b1, B_w2, B_b2, seg=A_seg_len)
```

```python
import functools

import jax
import jax.numpy as jnp
import numpy as np
from jax import lax
import jax.experimental.pallas as pl
import jax.experimental.pallas.tpu as pltpu

_LANES = 128
_WORDS = _LANES // 2
_EPS = 1e-5
_LOG2E = float(np.log2(np.e))
_F32 = jnp.float32
_BF16 = jnp.bfloat16
_U32 = jnp.uint32

_STEPS = 4
_RING = 8

CFG = dict(
    early_groups=12,
    columns="kqKQvV",
    mixer_done=48,
    sends=(16, 24, 28, 30, 31),
    load_order=(24, 25, 26, 27, 16, 17, 18, 19, 0, 1, 2, 7, 4, 5, 6, 3, 12, 13, 14, 15, 8, 9, 10, 23,
                40, 41, 42, 43, 28, 30, 29, 31, 32, 33, 34, 35, 20, 21, 22, 11, 36, 37, 38, 39, 44, 45, 46, 47),
    mlp_order=(24, 25, 26, 7, 0, 1, 30, 2, 14, 15, 19, 4, 5, 6, 9, 10, 3, 16, 17, 18,
               20, 8, 21, 22, 23, 28, 29, 31, 27, 11, 12, 13, 32, 33, 34, 35, 36, 37, 38, 39),
    a0=dict(qk=35, transpose=35, v=30, softmax=85, o=15, v_lag=10, head_start=3, burst=5, o_chunk=4, o_parts=2,
            mixer=(0, 0, 0, 48), mixer_split=96, tokens=(0, 32, 64, 96, 128), tiles=(0, 4, 9, 14, 14)),
    a2=dict(qk=20, transpose=35, v=40, softmax=75, o=15, v_lag=9, head_start=2, burst=5, o_chunk=4, o_parts=3,
            mixer=(0, 0, 0, 48), mixer_split=128, tokens=(0, 24, 64, 104, 128), tiles=(0, 0, 7, 14, 14), fast={}),
    a1=dict(qk=20, transpose=35, v=45, softmax=75, o=15, v_lag=12, head_start=4, burst=5, o_chunk=4, o_parts=2,
            mixer=(0, 0, 0, 48), mixer_split=128, tokens=(0, 24, 56, 96, 128), fast=dict(v=18)),
)

_METHOD = {1: ((1, 2, 3), (1, 3, 1)), 2: ((1, 1, 3), (-1, 3, 2)), 3: ((1, 2, 2), (1, 1, 1))}
_PAIR = {
    (1, 2): ((2, 1, 1), (-1, 1, 2), (0, -1, -1, 0, 0, 1, 1), (-1, 0, 0, 1, 1, 0, -1)),
    (1, 3): ((3, 1, 1), (1, 3, 2), (-1, 0, 0, -1, 1, 0, -1), (0, -1, -1, 0, 0, -1, 1)),
    (2, 3): ((3, -1, 2), (1, 3, 1), (-1, 0, -1, 0, 1, 0, 1), (0, 1, 0, -1, 0, 1, -1)),
}


def _hopcroft_kerr(methods, complete):
    prods = []

    def product(a_terms, x_terms):
        prods.append((tuple(a_terms), tuple(x_terms), {}))
        return len(prods) - 1

    def element(idx, m):
        return idx, m, [product([(1, fa, i) for i in idx], [(1, fx, i) for i in idx]) for _, fa, fx in _METHOD[m]]

    def pair(e, f):
        if e[1] > f[1]:
            both, fe, ef = pair(f, e)
            return both, ef, fe
        (fa, sa, fb), (sx, fx, fy), c_ef, c_fe = _PAIR[e[1], f[1]]
        both = element(e[0] + f[0], 6 - e[1] - f[1])
        cross = product([(1, fa, i) for i in e[0]] + [(sa, fb, i) for i in f[0]],
                        [(sx, fx, i) for i in e[0]] + [(1, fy, i) for i in f[0]])
        ids = e[2] + f[2] + both[2] + [cross]
        return both, dict(zip(ids, c_ef)), dict(zip(ids, c_fe))

    diag = [element((i,), m) for i, m in enumerate(methods)]
    y = {(i, i): {t: s for t, (s, _, _) in zip(e[2], _METHOD[e[1]])} for i, e in enumerate(diag)}
    merged = {}
    pairs = [(i, j) for i in range(len(methods)) for j in range(i + 1, len(methods))]
    for i, j in pairs:
        if methods[i] != methods[j]:
            merged[i, j], y[i, j], y[j, i] = pair(diag[i], diag[j])
    for i, j in pairs:
        if complete and methods[i] == methods[j]:
            k = i + 1
            _, ik_j, j_ik = pair(merged[i, k], diag[j])
            y[i, j] = {t: ik_j.get(t, 0) - y[k, j].get(t, 0) for t in sorted({*ik_j, *y[k, j]})}
            y[j, i] = {t: j_ik.get(t, 0) - y[j, k].get(t, 0) for t in sorted({*j_ik, *y[j, k]})}
    for ij, terms in y.items():
        for t, s in terms.items():
            if s:
                prods[t][2][ij] = s
    spare = [list(e[2]) for e in diag]
    quads = []
    for t in sorted(range(2 * len(diag), len(prods), 3), key=lambda t: sorted(i for _, _, i in prods[t][0])):
        owners = sorted(i for _, _, i in prods[t][0]) + list(range(len(diag)))
        quads += [t, t + 1, t + 2, next(spare[i] for i in owners if spare[i]).pop()]
    return [prods[t] for t in quads + sum(spare, [])]


_HK22 = _hopcroft_kerr((1, 2), True)
_HK55 = _hopcroft_kerr((1, 2, 3, 1, 2), True)
_HK56 = _hopcroft_kerr((1, 2, 3, 1, 2, 3), False)


def _signed_sum(terms):
    terms = sorted(terms, key=lambda t: -t[0])
    if terms[0][0] < 0:
        return -_signed_sum([(-s, v) for s, v in terms])
    acc = terms[0][1]
    for s, v in terms[1:]:
        acc = acc + v if s > 0 else acc - v
    return acc


def _left_factors(scheme, blocks):
    form = {}
    for j, (upper, lower) in enumerate(blocks):
        form[1, j], form[2, j], form[3, j] = upper, lower, upper + lower
    return [_signed_sum([(s, form[f, j]) for s, f, j in x]) for _, x, _ in scheme]


def _shared_pairs(sums):
    sums = [dict(y) for y in sums]
    while True:
        count = {}
        for y in sums:
            for a in y:
                for b in y:
                    if repr(a) < repr(b):
                        count[a, y[a] * y[b], b] = count.get((a, y[a] * y[b], b), 0) + 1
        best = max(count, key=count.get, default=None)
        if best is None or count[best] < 2:
            return sums
        a, s, b = best
        for y in sums:
            if a in y and b in y and y[a] * y[b] == s:
                y[best] = y.pop(a)
                del y[b]


def _store_right_factors(scheme, weight, dst):
    @functools.cache
    def term(key):
        if len(key) == 3:
            return _signed_sum([(1, term(key[0])), (key[1], term(key[2]))])
        return weight(*key).astype(_F32)

    for t, terms in enumerate(_shared_pairs([y for _, _, y in scheme])):
        if len(scheme[t][2]) > 1:
            dst(t)[...] = _signed_sum([(s, term(key)) for key, s in terms.items()]).astype(_BF16)


class _Collector:
    def __init__(self, scheme):
        self.scheme, self.pending, self.total, self.left = scheme, {}, {}, {}
        for a, _, _ in scheme:
            for _, _, i in a:
                self.left[i] = self.left.get(i, 0) + 1

    def add(self, t, product):
        for s, f, i in self.scheme[t][0]:
            self.pending.setdefault(i, {}).setdefault(f, []).append((s, product))
            self.left[i] -= 1
        done = []
        if t % 4 == 3 or t + 1 == len(self.scheme):
            for i, forms in self.pending.items():
                both = [(1, _signed_sum(forms[3]))] if 3 in forms else []
                for r, terms in enumerate((forms.get(1, []) + both, forms.get(2, []) + [(-s, v) for s, v in both])):
                    if (i, r) in self.total:
                        terms = terms + [(1, self.total[i, r])]
                    if terms:
                        self.total[i, r] = _signed_sum(terms)
                if self.left[i] == 0:
                    done.append((i, self.total.pop((i, 0)), self.total.pop((i, 1))))
            self.pending = {}
        return done


def _dot(a, b):
    return lax.dot_general(a, b, (((1,), (0,)), ((), ())), preferred_element_type=_F32)


def _rows(words):
    return pltpu.bitcast(words, _BF16)


def _center(x):
    inv_d = 1.0 / x.shape[-1]
    c = x - jnp.sum(x, axis=-1, keepdims=True) * inv_d
    return c, jnp.sum(c * c, axis=-1, keepdims=True) * inv_d


def _layernorm(x):
    c, v = _center(x)
    return c * lax.rsqrt(v + _EPS)


def _layernorm_twice(x):
    c, v = _center(x)
    r = lax.rsqrt(v + _EPS)
    return c * (r * lax.rsqrt(v * r * r + _EPS))


def _gelu(x):
    c = float(np.sqrt(2.0 / np.pi))
    half = 0.5 * x
    return half + half * jnp.tanh(x * (c + (0.044715 * c) * (x * x)))


def _column(vector):
    return jnp.broadcast_to(vector.astype(_F32).reshape(1, -1), (_LANES, vector.shape[0])).T


def _span(start, n, align):
    return pl.ds(start if isinstance(start, int) else pl.multiple_of(start, align), n)


def _lanes(j, n=1):
    return slice(j * _LANES, (j + n) * _LANES)


def _tile_words(j, n=1):
    return slice(j * _WORDS, (j + n) * _WORDS)


def _segment_order(n_heads, n_tiles, columns, plan, follows_projection, fast_qkv, fast_o):
    projections = []
    if fast_qkv:
        plan = {**plan, **plan["fast"]}
        last = {i: t | 3 for t, (a, _, _) in enumerate(_HK56) for _, _, i in a}
        for p in range(n_heads // 2):
            for t in range(len(_HK56)):
                made = [(m, 2 * p + b) for i, (m, b) in enumerate(columns) if last[i] == t]
                projections.append((("fast_qkv", p, t), 1, made))
    else:
        ahead = plan["head_start"] if follows_projection else 0
        projections += [(("start", m, h), n_tiles - 1, []) for h in range(ahead) for m in range(2)]
        for h in range(n_heads + plan["v_lag"]):
            if h < n_heads:
                n = 1 if h < ahead else n_tiles
                projections += [(("qkv", 1, h), n, [(1, h)]), (("qkv", 0, h), n, [(0, h)])]
            if h >= plan["v_lag"]:
                projections.append((("qkv", 2, h - plan["v_lag"]), n_tiles, [(2, h - plan["v_lag"])]))

    if fast_o:
        depth = n_heads // 5
        cuts = [c * depth // plan["o_parts"] for c in range(plan["o_parts"] + 1)]
        parts = [[(("fast_o", t, lo, hi), hi - lo, range(5 * lo, 5 * hi)) for t in range(len(_HK55))]
                 for lo, hi in zip(cuts, cuts[1:])]
        tail = [(("tail_o", c), 7 if c < 2 else 4, range(5 * depth, n_heads)) for c in range(3)]
        outputs = [sum(parts[:-1], []) + tail + parts[-1]]
    else:
        n = plan["o_chunk"]
        outputs = [[(("o", j, lo, lo + n), n, range(lo, lo + n)) for lo in range(0, n_heads, n)]
                   for j in range(n_tiles)]

    triples = [range(h, min(h + 3, n_heads)) for h in range(0, n_heads, 3)]
    attention = []
    for r in range(len(triples) + 2):
        new = triples[r] if r < len(triples) else ()
        old = triples[r - 2] if r >= 2 else ()
        keys = [((m, h), plan["qk"] + m * plan["transpose"]) for h in new for m in range(2)]
        values = [((2, h), plan["v"]) for h in old] + [(("p", r - 2), plan["softmax"])]
        if len(new) == len(old) == 3:
            attention.append((("values_rest", r - 2), values, [("rest", r - 2)]))
            attention += [(("both", r, c), keys + [(("rest", r - 2), 0)], [("o", old[c]), ("s", new[c])])
                          for c in range(3)]
            attention.append((("scores_rest", r), keys + [(("s", h), 0) for h in new], [("p", r)]))
        else:
            attention += [(("scores", r, c), keys, [("p", r)] * (h == new[-1])) for c, h in enumerate(new)]
            attention += [(("values", r - 2, c), values, [("o", h)]) for c, h in enumerate(old)]

    order, done, now, run = [], {}, 0, 0

    def wait(needs):
        return max(d - (now - done[key]) if key in done else np.inf for key, d in needs)

    while projections or attention or any(outputs):
        visit = min(attention, key=lambda v: max(wait(v[1]), 0), default=None)
        queue = min((q for q in outputs if q), key=lambda q: max(wait([(("o", h), plan["o"]) for h in q[0][2]]), 0))
        stuck = not projections and wait([(("o", h), 0) for h in queue[0][2]]) > 0
        if visit and (stuck or (run < plan["burst"] and wait(visit[1]) <= 0)):
            attention.remove(visit)
            op, n, made = visit[0], 1, visit[2]
            run += 1
        else:
            op, n, made = projections.pop(0) if projections else (*queue.pop(0)[:2], [])
            run = 0
        order.append(op)
        now += n
        for key in made:
            done[key] = now
    return order


def _kernel(x_hbm, mem0_hbm, wq_hbm, wk_hbm, wv_hbm, wo_hbm, w1t_hbm, b1_hbm, w2_hbm, b2_hbm, out_hbm,
            x_ref, first_ref, res_ref, out_ref, side_ref, mem0_ref, mem_ref,
            ring_ref, wqkv_ref, sum_qkv_ref, left_ref, early_ref, wo_ref, sum_o_ref, sum_tail_ref,
            w1t_ref, w2_ref, b1_ref, b2_ref, b1_col_ref, b2_col_ref, u_ref, hidden_ref, sum_act_ref,
            zero_ref, sems, ring_sems, w2_sems, *, cfg):
    S, D = res_ref.shape
    n_groups, G, _ = x_ref.shape
    n_early, seg, _ = first_ref.shape
    M = mem0_ref.shape[0]
    L = seg + M
    ride = seg - M
    _, H, _, Dh = wqkv_ref.shape
    F, F_pad = b1_ref.shape[0], w2_ref.shape[1]
    nd = D // _LANES
    n_pairs = H // 2
    depth = H // 5
    assert (nd, Dh, G, seg, M, H) == (5, _LANES, _LANES, _STEPS * M, 8, 32)
    assert sorted(cfg["load_order"]) == list(range(len(_HK56))) and sorted(cfg["mlp_order"]) == list(range(len(_HK55)))
    columns = [("qkv".index(c.lower()), int(c.isupper())) for c in cfg["columns"]]

    wqkv_words, sum_qkv_words, left_words, early_words, sum_o_words, sum_tail_words, hidden_words, sum_act_words = (
        ref.bitcast(_U32) for ref in (
            wqkv_ref, sum_qkv_ref, left_ref, early_ref, sum_o_ref, sum_tail_ref, hidden_ref, sum_act_ref))

    def put_tokens(lo, val):
        for j in range(nd):
            side_ref[pl.ds(j * G + lo, val.shape[0]), :] = pltpu.bitcast(val[:, _lanes(j)], _U32)

    def get_tokens(lo, n):
        return jnp.concatenate(
            [pltpu.bitcast(side_ref[_span(j * G + lo, n, 8), :], _F32) for j in range(nd)], axis=1)

    def side_words(j, word, n):
        return _span(nd * G + j * (S // 2) + word, n, 8)

    def qkv_left(upper, lower):
        blocks = [(upper[:, _lanes(j)], lower[:, _lanes(j)]) for j in range(nd)]
        blocks.append(tuple(_signed_sum([(-1, b[r]) for b in blocks]) for r in range(2)))
        return [left.astype(_BF16) for left in _left_factors(_HK56, blocks)]

    qkv_hbm_words = [w.bitcast(_U32) for w in (wq_hbm, wk_hbm, wv_hbm)]
    wo_hbm_words, w1t_hbm_words = wo_hbm.bitcast(_U32), w1t_hbm.bitcast(_U32)

    def pair_copies(*pairs):
        return [pltpu.make_async_copy(w.at[:, p, :], ring_ref.at[p & (_RING - 1), m], ring_sems.at[p & (_RING - 1)])
                for p in pairs for m, w in enumerate(qkv_hbm_words)]

    def wo_copy(j):
        return pltpu.make_async_copy(wo_hbm_words.at[:, :, _span(j * _LANES, _LANES, _LANES)], wo_ref.at[j], sems.at[3])

    def w2_copy(g):
        return pltpu.make_async_copy(w2_hbm.at[:, _span(g * G, G, G)], w2_ref.at[g & 1, pl.ds(0, F)], w2_sems.at[g & 1])

    def out_copy(row, n):
        return pltpu.make_async_copy(out_ref.at[pl.ds(row, n)], out_hbm.at[pl.ds(row, n)], sems.at[0])

    small_copies = [pltpu.make_async_copy(src, dst, sems.at[4]) for src, dst in (
        (x_hbm.at[0], x_ref.at[0]), (mem0_hbm, mem0_ref), (b1_hbm, b1_ref), (b2_hbm, b2_ref))]
    first_copy = pltpu.make_async_copy(x_hbm.at[pl.ds(0, n_early), pl.ds(0, seg), :], first_ref, sems.at[0])
    x1_copy = pltpu.make_async_copy(x_hbm.at[1], x_ref.at[1], sems.at[4])
    x_copy = pltpu.make_async_copy(x_hbm.at[pl.ds(2, n_groups - 2)], x_ref.at[pl.ds(2, n_groups - 2)], sems.at[1])
    w1_copies = [pltpu.make_async_copy(w1t_hbm_words.at[:, _lanes(k)], w1t_ref.at[k], sems.at[2])
                 for k in range(S // _LANES)]

    for c in small_copies + [first_copy] + pair_copies(0):
        c.start()
    for i in range(_STEPS):
        zero_ref[i] = 0
    w2_ref[:, F:F_pad, :] = jnp.zeros((2, F_pad - F, _LANES), _BF16)
    hidden_ref[:, F:F_pad, :] = jnp.zeros((nd, F_pad - F, _LANES), _BF16)
    for c in small_copies:
        c.wait()
    for c in pair_copies(1):
        c.start()
    b1_col_ref[...] = _column(b1_ref[...])
    b2_col_ref[...] = _column(b2_ref[...])
    x0 = x_ref[0, seg:G, :].astype(_F32)
    res_ref[seg:G, :] = x0
    put_tokens(seg, _layernorm(x0))
    first_copy.wait()
    for c in range(n_early // 2):
        upper, lower = (_layernorm(first_ref[c + r * n_early // 2].astype(_F32)) for r in range(2))
        for t, left in enumerate(qkv_left(upper, lower)):
            left_ref[t, c * seg:(c + 1) * seg, :] = left

    def prepare_pair(p):
        @functools.cache
        def weight(j, i):
            m, odd = columns[i]
            words = ring_ref[p & (_RING - 1), m, _lanes(j), :]
            return pltpu.bitcast(words & np.uint32(0xFFFF0000) if odd else words << 16, _F32)

        @functools.cache
        def rebased(j, i):
            skip = (i + 3) % 6
            if skip == nd:
                return 1, weight(j, i)
            return (-1, weight(skip, i)) if j == nd else (1, weight(j, i) - weight(skip, i))

        out = _Collector([_HK56[t] for t in cfg["load_order"]])
        for n, t in enumerate(cfg["load_order"]):
            sum_qkv_ref[p, t] = _signed_sum(
                [(s * rebased(j, i)[0], rebased(j, i)[1]) for (i, j), s in _HK56[t][2].items()]).astype(_BF16)
            for i, upper, lower in out.add(n, _dot(_rows(left_words[t]), _rows(sum_qkv_words[p, t]))):
                m, odd = columns[i]
                early_ref[m, 2 * p + odd] = jnp.concatenate([upper, lower], axis=0).astype(_BF16)
        for i, (m, odd) in enumerate(columns):
            for j in range(nd):
                wqkv_ref[m, 2 * p + odd, _lanes(j), :] = weight(j, i).astype(_BF16)

    def prepare_pairs(it, carry):
        p, last = 2 * it, n_pairs // 2 - 1
        for c in pair_copies(p, p + 1):
            c.wait()

        @pl.when(it + 2 <= last)
        def _():
            for c in pair_copies(p + 4, p + 5):
                c.start()

        @pl.when((it >= last - nd) & (it < last))
        def _():
            wo_copy(it - (last - nd)).start()

        @pl.when(it == last)
        def _():
            x1_copy.start()
            w2_copy(0).start()

        prepare_pair(p)
        prepare_pair(p + 1)
        return carry

    def prepare_wo(i, carry):
        block, words, rows = i >> 3, _span((i & 7) * 8, 8, 8), _span(i * 16, 16, 16)
        _store_right_factors(_HK55, lambda a, b: _rows(wo_ref[a, 5 * block + b, words, :]),
                             lambda t: sum_o_ref.at[t, rows])
        return carry

    for p in range(2):
        for c in pair_copies(p):
            c.wait()
        for c in pair_copies(2 * p + 2, 2 * p + 3):
            c.start()
        prepare_pair(p)
    lax.fori_loop(1, n_pairs // 2, prepare_pairs, 0)
    for j in range(nd):
        wo_copy(j).wait()
    lax.fori_loop(0, depth * 8, prepare_wo, 0)
    for c in range(2):
        _store_right_factors(_HK22, lambda a, b: _rows(wo_ref[2 * c + a, 5 * depth + b]),
                             lambda t: sum_tail_ref.at[c, t])
    x1_copy.wait()
    for c in [x_copy] + w1_copies:
        c.start()

    def residual(layer, g, lo, hi, cols=slice(None)):
        if layer == 1:
            return res_ref[_span(g * G + lo, hi - lo, 8), cols]
        lo16 = lo // 16 * 16
        return x_ref[g, lo16:-(-hi // 16) * 16, cols].astype(_F32)[lo - lo16:hi - lo16]

    def mixer_input(g, lo, hi):
        h = _layernorm_twice(res_ref[_span(g * G + lo, hi - lo, 8), :]).astype(_BF16)
        for j in range(nd):
            side_ref[side_words(j, g * (G // 2) + lo // 2, (hi - lo) // 2), :] = pltpu.bitcast(h[:, _lanes(j)], _U32)

    def wo_tiles(j, heads):
        return _rows(jnp.concatenate([wo_ref[j, h] for h in heads], axis=0))

    def attend_group(layer, fast, plan, g, carry):
        row = lax.broadcasted_iota(jnp.int32, (L, _LANES), 0)
        lane = lax.broadcasted_iota(jnp.int32, (L, _LANES), 1)
        key = lane - jnp.where(lane < L, 0, jnp.where(lane < 2 * L, L, 2 * L))
        visible = ((key <= row) | (key >= seg) | (row >= seg)) & (key < L)
        hidden = jnp.where(key < L, -1e9 * _LOG2E, -jnp.inf).astype(_F32)

        @functools.cache
        def window(c, n=L):
            return (lane[0:n] >= c * L) & (lane[0:n] < (c + 1) * L)

        def by_window(parts):
            out = parts[-1]
            for c in reversed(range(len(parts) - 1)):
                out = jnp.where(window(c), parts[c], out)
            return out

        def by_rows(piece):
            rows = [slice(c * L, min((c + 1) * L, _LANES)) for c in range(4)]
            return jnp.concatenate([piece(c, r) for c, r in enumerate(rows)], axis=0).astype(_BF16)

        def diagonal(tile):
            return by_rows(lambda c, r: jnp.where(window(c), tile[r], 0.0) if c < 3 else jnp.zeros_like(tile[r]))

        def softmax(scores):
            t = jnp.where(visible, scores * (Dh ** -0.5 * _LOG2E), hidden)
            top = by_window([jnp.max(jnp.where(window(c), t, -jnp.inf), axis=-1, keepdims=True) for c in range(3)])
            ex = jnp.exp2(t - top)
            z = by_window([jnp.sum(jnp.where(window(c), ex, 0.0), axis=-1, keepdims=True) for c in range(3)])
            r = pl.reciprocal(z, approx=True)
            return ex * (r * (2.0 - z * r))

        if layer == 0:
            @pl.when(g == 1)
            def _():
                x_copy.wait()

            w2_copy(g).wait()

            @pl.when(g + 1 < n_groups)
            def _():
                w2_copy(g + 1).start()

        ahead = {}
        behind = {}
        g_prev, g_next = jnp.maximum(g - 1, 0), jnp.minimum(g + 1, n_groups - 1)

        for step in range(_STEPS):
            fast_qkv, fast_o = fast and step == 0, step == _STEPS - 1
            started, qkv, part, p, o, acc = {}, {}, {}, {}, {}, {}
            riders = get_tokens(seg + step * ride + (zero_ref[step] if step else 0), ride)
            carried = jnp.concatenate([riders, mem_ref[...]], axis=0)
            if fast_qkv:
                left = qkv_left(get_tokens(0, seg), carried)

            if step < 2:
                lo, hi = (cfg["mixer_done"], plan["mixer_split"], G)[step:step + 2]
                if hi > lo:
                    mixer_input(g_prev, lo, hi)
            if step and plan["mixer"][step] > plan["mixer"][step - 1]:
                assert plan["mixer"][step] <= step * ride
                mixer_input(g, *plan["mixer"][step - 1:step + 1])
            lo, hi = max(plan["tokens"][step], 0 if fast else seg), plan["tokens"][step + 1]
            if hi > lo:
                assert hi <= seg + (step + 1) * ride
                put_tokens(lo, _layernorm(residual(layer, g_next, lo, hi)))
            if layer == 0:
                for k in range(*plan["tiles"][step:step + 2]):
                    w = w2_ref[g & 1, _lanes(k), :].T
                    side_ref[side_words(nd + k, g * (G // 2), G // 2), :] = pltpu.bitcast(w, _U32)

            @functools.cache
            def carried_columns(lo, hi):
                return carried[:, _lanes(lo, hi - lo)].astype(_BF16)

            def project(m, h, lo, hi):
                return _dot(carried_columns(lo, hi), _rows(wqkv_words[m, h, _tile_words(lo, hi - lo), :]))

            @functools.cache
            def outputs(lo, hi):
                return jnp.concatenate([o[h] for h in range(lo, hi)], axis=1).astype(_BF16)

            def projected(m, h, tokens, y):
                tokens = jnp.concatenate([tokens, y[0:ride]], axis=0)
                qkv[m, h] = jnp.concatenate([tokens[0:seg], y[ride:seg]], axis=0)
                if step + 1 < _STEPS:
                    ahead[m, h] = tokens[seg:]

            @functools.cache
            def stacked(m, r):
                rows = [qkv[m, h] for h in range(3 * r, min(3 * r + 3, H))]
                rows.append(jnp.zeros((_LANES - len(rows) * L, Dh), _F32))
                tile = jnp.concatenate(rows, axis=0)
                return tile.T if m == 1 else tile

            def attended(h, y):
                tokens = y[0:seg] if step == 0 else jnp.concatenate([behind.pop(h), y[0:seg]], axis=0)
                o[h] = jnp.concatenate([y[seg:L], tokens[0:ride]], axis=0)
                behind[h] = tokens[ride:]

            def finish(j, tokens, mem):
                mem_ref[:, _lanes(j)] = mem
                res_ref[_span(g * G + step * ride, tokens.shape[0], 8), _lanes(j)] = tokens

            for kind, *arg in _segment_order(H, nd, columns, plan, step > 0, fast_qkv, fast_o):
                if kind == "start":
                    started[tuple(arg)] = project(*arg, 0, nd - 1)
                elif kind == "qkv":
                    m, h = arg
                    y = project(m, h, nd - 1, nd) + started.pop((m, h)) if (m, h) in started else project(m, h, 0, nd)
                    if step:
                        tokens = ahead.pop((m, h))
                    else:
                        tokens = _rows(early_words[m, h, _span(g * (seg // 2), seg // 2, 8), :]).astype(_F32)
                    projected(m, h, tokens, y)
                elif kind == "fast_qkv":
                    pair, t = arg
                    if t == 0:
                        out = _Collector(_HK56)
                    for i, upper, lower in out.add(t, _dot(left[t], _rows(sum_qkv_words[pair, t]))):
                        projected(columns[i][0], 2 * pair + columns[i][1], upper, lower)
                elif kind == "scores":
                    r, c = arg
                    part.setdefault(r, []).append(_dot(qkv[0, 3 * r + c], stacked(1, r).astype(_BF16)))
                    if c == 2 or 3 * r + c == H - 1:
                        p[r] = softmax(by_window(part.pop(r)))
                elif kind == "values":
                    r, c = arg
                    attended(3 * r + c, _dot(jnp.where(window(c), p[r], 0.0), stacked(2, r).astype(_BF16)))
                elif kind == "both":
                    r, c = arg
                    tile = by_rows(lambda d, rows: jnp.where(window(c), 0.0, stacked(2, r - 2)[rows]) if d == c
                                   else jnp.where(window(c, rows.stop - rows.start), stacked(1, r)[rows], 0.0))
                    y = _dot(jnp.where(window(c), p[r - 2], qkv[0, 3 * r + c]), tile)
                    part.setdefault(r, []).append(y)
                    attended(3 * (r - 2) + c, jnp.where(window(c), part["values_rest", r - 2], y))
                elif kind == "values_rest":
                    part[kind, arg[0]] = _dot(p[arg[0]], diagonal(stacked(2, arg[0])))
                elif kind == "scores_rest":
                    r, = arg
                    y = _dot(by_window([qkv[0, 3 * r + c] for c in range(3)]), diagonal(stacked(1, r)))
                    p[r] = softmax(by_window(part.pop(r)) + y)
                elif kind == "o":
                    j, lo, hi = arg
                    if lo == 0:
                        tokens = residual(layer, g, step * ride, (step + 1) * ride, _lanes(j))
                        acc[j] = jnp.concatenate([jnp.zeros((M, _LANES), _F32), tokens], axis=0)
                    acc[j] = _dot(outputs(lo, hi), wo_tiles(j, range(lo, hi))) + acc[j]
                    if hi == H:
                        finish(j, acc[j][M:], acc[j][0:M])
                elif kind == "tail_o":
                    c, = arg
                    blocks = [(o[h], behind[h]) for h in range(5 * depth, H)]
                    if c < 2:
                        tail = _Collector(_HK22)
                        for t, lhs in enumerate(_left_factors(_HK22, blocks)):
                            ((i, j), s), *more = _HK22[t][2].items()
                            if more:
                                y = _dot(lhs, _rows(sum_tail_words[c, t]))
                            else:
                                y = _dot(lhs if s > 0 else -lhs, wo_tiles(2 * c + i, [5 * depth + j]))
                            for i, upper, lower in tail.add(t, y):
                                acc["tail", 2 * c + i] = (upper, lower)
                    else:
                        lhs = jnp.concatenate([jnp.concatenate(b, axis=0) for b in blocks], axis=1)
                        y = _dot(lhs, wo_tiles(nd - 1, range(5 * depth, H)))
                        acc["tail", nd - 1] = (y[0:seg], y[seg:])
                elif kind == "fast_o":
                    t, lo, hi = arg
                    if t == 0:
                        out = _Collector(_HK55)
                        lefts = [_left_factors(_HK55, [(o[h], behind[h]) for h in range(5 * c, 5 * c + 5)])
                                 for c in range(lo, hi)]
                    lhs = jnp.concatenate([factors[t] for factors in lefts], axis=1)
                    ((i, j), s), *more = _HK55[t][2].items()
                    if more:
                        y = _dot(lhs, _rows(sum_o_words[t, _tile_words(lo, hi - lo), :]))
                    else:
                        y = _dot(lhs if s > 0 else -lhs, wo_tiles(i, [5 * c + j for c in range(lo, hi)]))
                    if lo > 0:
                        y = y + acc.pop(t)
                    if hi < depth:
                        acc[t] = y
                    else:
                        for i, upper, lower in out.add(t, y):
                            upper, lower = upper + acc["tail", i][0], lower + acc["tail", i][1]
                            tokens = jnp.concatenate([upper[M:], lower], axis=0)
                            finish(i, tokens + residual(layer, g, step * ride, G, _lanes(i)), upper[0:M])
        return carry

    def token_matmul(n_rows, nk, weights, acts, seed, emit, chunk_done):
        deep, rest = divmod(nk, 5)
        plans = [(_HK22, 2, 2 * c, 5 * deep, rest // 2, len(_HK55) * deep + len(_HK22) * c * (rest // 2))
                 for c in range(2 if rest > 1 else 0)]
        plans.append((_HK55, 5, 0, 0, deep, 0))

        def lead(it, carry):
            for word in (it * 16, it * 16 + 8):
                rows = _span(2 * word, 16, 16)
                for scheme, size, j0, k0, m, t0 in plans:
                    for c in range(m):
                        _store_right_factors(scheme, lambda a, b: acts(k0 + size * c + b, j0 + a, word, 8),
                                             lambda t: sum_act_ref.at[t0 + t * m + c, rows])
            n = n_rows // 4
            lhs = jnp.concatenate([weights(it * (n // 2), n // 2, k) for k in range(5 * deep, nk)], axis=1)
            for j in range(2 * len(plans) - 2, nd):
                rhs = jnp.concatenate([acts(k, j, 0, _WORDS) for k in range(5 * deep, nk)], axis=0)
                seed(_span(it * n, n, 16), j, _dot(lhs, rhs))
            return carry

        lax.fori_loop(0, 4, lead, 0)

        @functools.cache
        def right(plan, t):
            scheme, size, j0, k0, m, t0 = plans[plan]
            ((i, j), s), *more = scheme[t][2].items()
            if more:
                return 1, jnp.concatenate([_rows(sum_act_words[t0 + t * m + c]) for c in range(m)], axis=0)
            return s, jnp.concatenate([acts(k0 + size * c + j, j0 + i, 0, _WORDS) for c in range(m)], axis=0)

        for row in range(0, n_rows, 2 * seg):
            @functools.cache
            def half(f, block):
                return jnp.concatenate([weights((row + (f - 1) * seg) // 2, seg // 2, k) for k in block], axis=1)

            @functools.cache
            def form(f, block):
                return form(1, block) + form(2, block) if f == 3 else half(f, block).astype(_F32)

            extra = {}
            for plan, (scheme, size, j0, k0, m, _) in enumerate(plans):
                order = cfg["mlp_order"] if scheme is _HK55 else range(len(scheme))
                out = _Collector([scheme[t] for t in order])
                blocks = [range(k0 + j, k0 + size * m, size) for j in range(size)]
                for n, t in enumerate(order):
                    x = scheme[t][1]
                    s, rhs = right(plan, t)
                    if len(x) == 1 and x[0][1] < 3 and s > 0:
                        lhs = half(x[0][1], blocks[x[0][2]])
                    else:
                        lhs = _signed_sum([(s * sx, form(f, blocks[j])) for sx, f, j in x])
                    for i, upper, lower in out.add(n, _dot(lhs, rhs)):
                        val = jnp.concatenate([upper, lower], axis=0)
                        if scheme is _HK55:
                            emit(slice(row, row + 2 * seg), i, val + extra.pop(i) if i in extra else val)
                        else:
                            extra[j0 + i] = val
            chunk_done(row // (2 * seg) + 1)

    def seed_hidden(rows, j, u):
        u_ref[rows, _lanes(j)] = u + b1_col_ref[rows, :]

    def emit_hidden(rows, j, u):
        hidden_ref[j, rows, :] = _gelu(u + u_ref[rows, _lanes(j)]).astype(_BF16)

    def seed_output(rows, j, y):
        res_ref[rows, _lanes(j)] = res_ref[rows, _lanes(j)] + y

    def emit_output(layer, rows, j, y):
        x = res_ref[rows, _lanes(j)] + (y + b2_col_ref[rows, :])
        if layer == 0:
            res_ref[rows, _lanes(j)] = x
        else:
            out_ref[rows, _lanes(j)] = x.astype(_BF16)

    def send_output(layer, chunks):
        cuts = (0, *cfg["sends"], S // (2 * seg))
        if layer == 1 and chunks in cuts:
            sent = cuts[cuts.index(chunks) - 1]
            out_copy(sent * 2 * seg, (chunks - sent) * 2 * seg).start()

    def attend(layer, fast, plan, lo, hi):
        lax.fori_loop(lo, hi, functools.partial(attend_group, layer, fast, plan), 0)

    for layer in range(2):
        mem_ref[...] = mem0_ref[...].astype(_F32)
        if layer == 0:
            attend(0, False, cfg["a0"], 0, n_early)
            put_tokens(0, _layernorm(residual(0, n_early, 0, seg)))
            attend(0, True, cfg["a2"], n_early, n_groups)
            for c in w1_copies:
                c.wait()
        else:
            put_tokens(0, _layernorm(residual(1, 0, 0, G)))
            attend(1, True, cfg["a1"], 0, n_groups)
        mixer_input(n_groups - 1, cfg["mixer_done"], G)
        token_matmul(F, S // _LANES,
                     lambda word, n, k: _rows(w1t_ref[k, _span(word, n, 8), :]),
                     lambda k, j, word, n: _rows(side_ref[side_words(j, k * _WORDS + word, n), :]),
                     seed_hidden, emit_hidden, lambda chunks: None)
        token_matmul(S, F_pad // _LANES,
                     lambda word, n, k: _rows(side_ref[side_words(nd + k, word, n), :]),
                     lambda k, j, word, n: _rows(hidden_words[j, _span(k * _WORDS + word, n, 8), :]),
                     seed_output, functools.partial(emit_output, layer), functools.partial(send_output, layer))
    out_copy(0, S).wait()


def build(cfg, x, mem0, wq, wk, wv, wo, w1, b1, w2, b2, seg=32):
    _, S, D = x.shape
    M = mem0.shape[1]
    _, H, Dh = wq.shape
    F = w1.shape[1]
    F_pad = pl.cdiv(F, _LANES) * _LANES
    G = _STEPS * seg
    nd, n_early = D // _LANES, cfg["early_groups"]
    hbm = pl.BlockSpec(memory_space=pltpu.HBM)
    out = pl.pallas_call(
        functools.partial(_kernel, cfg=cfg),
        out_shape=jax.ShapeDtypeStruct((S, D), x.dtype),
        in_specs=[hbm] * 10,
        out_specs=hbm,
        scratch_shapes=[
            pltpu.VMEM((S // G, G, D), _BF16),
            pltpu.VMEM((n_early, seg, D), _BF16),
            pltpu.VMEM((S, D), _F32),
            pltpu.VMEM((S, D), _BF16),
            pltpu.VMEM((nd * G + (D + F_pad) // _LANES * S // 2, _LANES), _U32),
            pltpu.VMEM((M, D), _BF16),
            pltpu.VMEM((M, D), _F32),
            pltpu.VMEM((_RING, 3, D, Dh), _U32),
            pltpu.VMEM((3, H, D, Dh), _BF16),
            pltpu.VMEM((H // 2, len(_HK56), _LANES, Dh), _BF16),
            pltpu.VMEM((len(_HK56), n_early * seg // 2, _LANES), _BF16),
            pltpu.VMEM((3, H, n_early * seg, Dh), _BF16),
            pltpu.VMEM((nd, H, _WORDS, _LANES), _U32),
            pltpu.VMEM((len(_HK55), H // 5 * _LANES, _LANES), _BF16),
            pltpu.VMEM((2, len(_HK22), _LANES, _LANES), _BF16),
            pltpu.VMEM((S // _LANES, F // 2, _LANES), _U32),
            pltpu.VMEM((2, F_pad, G), _BF16),
            pltpu.VMEM((F,), _BF16),
            pltpu.VMEM((S,), _BF16),
            pltpu.VMEM((F, _LANES), _F32),
            pltpu.VMEM((S, _LANES), _F32),
            pltpu.VMEM((F, D), _F32),
            pltpu.VMEM((nd, F_pad, _LANES), _BF16),
            pltpu.VMEM((3 * len(_HK55), _LANES, _LANES), _BF16),
            pltpu.SMEM((_STEPS,), jnp.int32),
            pltpu.SemaphoreType.DMA((5,)),
            pltpu.SemaphoreType.DMA((_RING,)),
            pltpu.SemaphoreType.DMA((2,)),
        ],
        compiler_params=pltpu.CompilerParams(
            vmem_limit_bytes=124 * 1024 * 1024,
            flags={"XLA_TPU_EVENLY_DISTRIBUTE_CRITICAL_NODES": True}),
        name="fused",
    )(x.reshape(S // G, G, D), mem0.reshape(M, D), wq, wk, wv, wo, w1.T, b1, w2, b2)
    return out.reshape(x.shape)


@functools.partial(jax.jit, static_argnames=("A_seg_len",))
def pallas_interleave_layers__memory_aug_recurrent_mem_tr__mixer_token_mlp__prompt_kernel(
    A_x: jax.Array,
    A_mem0: jax.Array,
    A_Wq: jax.Array,
    A_Wk: jax.Array,
    A_Wv: jax.Array,
    A_Wo: jax.Array,
    A_seg_len: int,
    B_x: jax.Array,
    B_w1: jax.Array,
    B_b1: jax.Array,
    B_w2: jax.Array,
    B_b2: jax.Array,
):
    del B_x
    return build(CFG, A_x, A_mem0, A_Wq, A_Wk, A_Wv, A_Wo, B_w1, B_b1, B_w2, B_b2, seg=A_seg_len)
```
